```python
import os as _os
_os.environ.setdefault("JAX_PLATFORMS", "cpu")
import jax
import jax.numpy as jnp

def _softmax(x, axis=-1):
    return jax.nn.softmax(x, axis=axis)
def _gelu(x):
    return jax.nn.gelu(x, approximate=True)
def _silu(x):
    return jax.nn.silu(x)
def _sigmoid(x):
    return jax.nn.sigmoid(x)
def _layernorm(x, axis=-1, eps=1e-5):
    m = jnp.mean(x, axis=axis, keepdims=True)
    v = jnp.var(x, axis=axis, keepdims=True)
    return (x - m) / jnp.sqrt(v + eps)
def _scatter_add(tgt, idx, src, axis=0):
    return tgt.at[idx].add(src)
def _segment_sum(src, seg, n):
    return jax.ops.segment_sum(src, seg, n)
class _Rng:
    def __init__(self, key):
        self._k = key
    def _next(self):
        self._k, sub = jax.random.split(self._k)
        return sub
    def normal(self, shape):
        return jax.random.normal(self._next(), shape, dtype=jnp.bfloat16)
    def randint(self, lo, hi, shape):
        return jax.random.randint(self._next(), shape, lo, hi, dtype=jnp.int32)
    def uniform(self, shape, lo=0.0, hi=1.0):
        return jax.random.uniform(self._next(), shape, jnp.bfloat16, lo, hi)
    def permutation(self, n):
        return jax.random.permutation(self._next(), n)


kernel_name = 'standalone__dense_activation_gelu__prompt'

def setup_inputs():
    _rng = _Rng(jax.random.key(int.from_bytes(__import__("os").urandom(4), "little")))
    _w = (lambda a: (lambda t: t.astype(jnp.bfloat16) if jnp.issubdtype(t.dtype, jnp.floating) else t)(jnp.asarray(a)))
    B, S, D, F = 1, 2048, 640, 1728
    return {
        "x": _w((lambda *s: _rng.normal(s) * 0.05)(B, S, D)),
        "w1": _w((lambda *s: _rng.normal(s) * 0.05)(D, F) * (D ** -0.5)),
        "b1": _w((lambda *s: _rng.normal(s) * 0.05)(F) * 0.01),
        "w2": _w((lambda *s: _rng.normal(s) * 0.05)(F, D) * (F ** -0.5)),
        "b2": _w((lambda *s: _rng.normal(s) * 0.05)(D) * 0.01),
    }

def reference(x, w1, b1, w2, b2):
    h = jnp.einsum("bsd,df->bsf", x, w1) + b1
    h = _gelu(h)
    return jnp.einsum("bsf,fd->bsd", h, w2) + b2
```

```python
import functools
import jax
import jax.numpy as jnp
import jax.experimental.pallas as pl
import jax.experimental.pallas.tpu as pltpu

TM = 256

def _gelu_tanh(h):
    c0 = 0.7978845608028654
    c1 = 0.044715 * c0
    inner = h * (c0 + c1 * (h * h))
    return 0.5 * h * (1.0 + jnp.tanh(inner))

def _kernel(x_ref, w1_ref, b1_ref, w2_ref, b2_ref, o_ref):
    x = x_ref[...]
    h = jnp.dot(x, w1_ref[...], preferred_element_type=jnp.float32)
    h = h + b1_ref[...].astype(jnp.float32)
    g = _gelu_tanh(h).astype(jnp.bfloat16)
    o = jnp.dot(g, w2_ref[...], preferred_element_type=jnp.float32)
    o = o + b2_ref[...].astype(jnp.float32)
    o_ref[...] = o.astype(o_ref.dtype)

@jax.jit
def pallas_standalone__dense_activation_gelu__prompt_kernel(x, w1, b1, w2, b2):
    B, S, D = x.shape
    F = w1.shape[1]
    M = B * S
    x2 = x.reshape(M, D)
    b1r = b1.reshape(1, F)
    b2r = b2.reshape(1, D)
    out = pl.pallas_call(
        _kernel,
        grid=(M // TM,),
        in_specs=[
            pl.BlockSpec((TM, D), lambda i: (i, 0)),
            pl.BlockSpec((D, F), lambda i: (0, 0)),
            pl.BlockSpec((1, F), lambda i: (0, 0)),
            pl.BlockSpec((F, D), lambda i: (0, 0)),
            pl.BlockSpec((1, D), lambda i: (0, 0)),
        ],
        out_specs=pl.BlockSpec((TM, D), lambda i: (i, 0)),
        out_shape=jax.ShapeDtypeStruct((M, D), jnp.bfloat16),
        compiler_params=pltpu.CompilerParams(
            dimension_semantics=("arbitrary",),
            vmem_limit_bytes=100 * 1024 * 1024,
        ),
    )(x2, w1, b1r, w2, b2r)
    return out.reshape(B, S, D)
```

```python
import functools
import jax
import jax.numpy as jnp
from jax import lax
import jax.experimental.pallas as pl
import jax.experimental.pallas.tpu as pltpu

R0 = 512
W1_BOUNDS = (0, 256, 768, 1728)
RA = 512
RB = 512
NBW = 128

_NT = (((1,), (1,)), ((), ()))


def _gelu_tanh(h):
    c0 = 0.7978845608028654
    c1 = 0.044715 * c0
    inner = h * (c0 + c1 * (h * h))
    return 0.5 * h * (1.0 + jnp.tanh(inner))


def _make_kernel(M, D, F):
    nc1 = len(W1_BOUNDS) - 1
    nb_cnt = D // NBW
    rb_cnt = M // RB
    n_out = nb_cnt * rb_cnt

    def kernel(x_hbm, w1t_hbm, b1_hbm, w2_hbm, b2_hbm, o_hbm,
               x_buf, w1_buf, w2_buf, b1_buf, b2_buf, g_buf, o_buf,
               x_sem, w1_sem, w2_sem, b_sem, o_sem):
        def x_copy(k):
            r0, r1 = (0, R0) if k == 0 else (R0, M)
            return pltpu.make_async_copy(
                x_hbm.at[pl.ds(r0, r1 - r0)], x_buf.at[pl.ds(r0, r1 - r0)],
                x_sem.at[k])

        def w1_copy(c):
            r0, r1 = W1_BOUNDS[c], W1_BOUNDS[c + 1]
            return pltpu.make_async_copy(
                w1t_hbm.at[pl.ds(r0, r1 - r0)], w1_buf.at[pl.ds(r0, r1 - r0)],
                w1_sem.at[c])

        def w2_copy():
            return pltpu.make_async_copy(w2_hbm, w2_buf, w2_sem.at[0])

        def b1_copy():
            return pltpu.make_async_copy(b1_hbm, b1_buf, b_sem.at[0])

        def b2_copy():
            return pltpu.make_async_copy(b2_hbm, b2_buf, b_sem.at[1])

        def o_copy(rb, nb):
            return pltpu.make_async_copy(
                o_buf.at[pl.ds(rb * RB, RB), pl.ds(nb * NBW, NBW)],
                o_hbm.at[pl.ds(rb * RB, RB), pl.ds(nb * NBW, NBW)],
                o_sem.at[rb * nb_cnt + nb])

        b1_copy().start()
        b2_copy().start()
        w1_copy(0).start()
        x_copy(0).start()
        for c in range(1, nc1):
            w1_copy(c).start()
        x_copy(1).start()
        w2_copy().start()

        x_copy(0).wait()
        b1_copy().wait()
        b1 = b1_buf[...].reshape(1, F).astype(jnp.float32)
        for c in range(nc1):
            c0, c1 = W1_BOUNDS[c], W1_BOUNDS[c + 1]
            w1_copy(c).wait()
            h = lax.dot_general(x_buf[0:R0, :], w1_buf[c0:c1, :], _NT,
                                preferred_element_type=jnp.float32)
            g_buf[0:R0, c0:c1] = _gelu_tanh(h + b1[:, c0:c1]).astype(jnp.bfloat16)

        x_copy(1).wait()
        for r0 in range(R0, M, RA):
            h = lax.dot_general(x_buf[r0:r0 + RA, :], w1_buf[...], _NT,
                                preferred_element_type=jnp.float32)
            g_buf[r0:r0 + RA, :] = _gelu_tanh(h + b1).astype(jnp.bfloat16)

        w2_copy().wait()
        b2_copy().wait()
        b2 = b2_buf[...].reshape(1, D).astype(jnp.float32)
        for nb in range(nb_cnt):
            n0 = nb * NBW
            for rb in range(rb_cnt):
                r0 = rb * RB
                o = jnp.dot(g_buf[r0:r0 + RB, :], w2_buf[:, n0:n0 + NBW],
                            preferred_element_type=jnp.float32)
                o_buf[r0:r0 + RB, n0:n0 + NBW] = (
                    o + b2[:, n0:n0 + NBW]).astype(o_buf.dtype)
                o_copy(rb, nb).start()

        for nb in range(nb_cnt):
            for rb in range(rb_cnt):
                o_copy(rb, nb).wait()

    return kernel, nc1, n_out


@jax.jit
def pallas_standalone__dense_activation_gelu__prompt_kernel(x, w1, b1, w2, b2):
    B, S, D = x.shape
    F = w1.shape[1]
    M = B * S
    x2 = x.reshape(M, D)
    w1t = w1.T
    kernel, nc1, n_out = _make_kernel(M, D, F)
    any_spec = pl.BlockSpec(memory_space=pl.ANY)
    out = pl.pallas_call(
        kernel,
        in_specs=[any_spec] * 5,
        out_specs=any_spec,
        out_shape=jax.ShapeDtypeStruct((M, D), jnp.bfloat16),
        scratch_shapes=[
            pltpu.VMEM((M, D), jnp.bfloat16),
            pltpu.VMEM((F, D), jnp.bfloat16),
            pltpu.VMEM((F, D), jnp.bfloat16),
            pltpu.VMEM((F,), jnp.bfloat16),
            pltpu.VMEM((D,), jnp.bfloat16),
            pltpu.VMEM((M, F), jnp.bfloat16),
            pltpu.VMEM((M, D), jnp.bfloat16),
            pltpu.SemaphoreType.DMA((2,)),
            pltpu.SemaphoreType.DMA((nc1,)),
            pltpu.SemaphoreType.DMA((1,)),
            pltpu.SemaphoreType.DMA((2,)),
            pltpu.SemaphoreType.DMA((n_out,)),
        ],
        compiler_params=pltpu.CompilerParams(
            vmem_limit_bytes=100 * 1024 * 1024,
        ),
    )(x2, w1t, b1, w2, b2)
    return out.reshape(B, S, D)
```

```python
import jax
import jax.numpy as jnp
from jax import lax
import jax.experimental.pallas as pl
import jax.experimental.pallas.tpu as pltpu

_LANE = 128
_ROW_CHUNK = 512
_BF16_SUBLANES = 16

_NT = (((1,), (1,)), ((), ()))


def _gelu_tanh(h):
    c0 = 0.7978845608028654
    c1 = 0.044715 * c0
    inner = h * (c0 + c1 * (h * h))
    return 0.5 * h * (1.0 + jnp.tanh(inner))


def _make_plan(M, D, F):
    assert M % _ROW_CHUNK == 0 and M >= 2 * _ROW_CHUNK, M
    assert D % _LANE == 0, D
    assert F % _BF16_SUBLANES == 0 and F >= 8 * _LANE, F
    r_early = _ROW_CHUNK
    x_rows = ((0, r_early // 2), (r_early // 2, r_early), (r_early, M))
    w1_bounds = (0, 2 * _LANE, 6 * _LANE, F)
    rest_chunks = (_ROW_CHUNK,) * ((M - r_early) // _ROW_CHUNK)
    return r_early, x_rows, w1_bounds, rest_chunks


def _make_kernel(M, D, F):
    r_early, x_rows, w1_bounds, rest_chunks = _make_plan(M, D, F)
    n_x = len(x_rows)
    n_w1 = len(w1_bounds) - 1
    n_cb = D // _LANE
    n_rb = M // _ROW_CHUNK
    f_main = (F // _LANE) * _LANE

    def kernel(x_hbm, w1t_hbm, b1_hbm, w2_hbm, b2_hbm, o_hbm,
               x_buf, w1_buf, w2_buf, b1_buf, b2_buf, g_buf, o_buf,
               x_sem, w1_sem, w2_sem, b_sem, o_sem):

        def x_copy(k):
            r0, r1 = x_rows[k]
            return pltpu.make_async_copy(
                x_hbm.at[pl.ds(r0, r1 - r0)], x_buf.at[pl.ds(r0, r1 - r0)],
                x_sem.at[k])

        def w1_copy(c):
            r0, r1 = w1_bounds[c], w1_bounds[c + 1]
            return pltpu.make_async_copy(
                w1t_hbm.at[pl.ds(r0, r1 - r0)], w1_buf.at[pl.ds(r0, r1 - r0)],
                w1_sem.at[c])

        def w2_copy():
            return pltpu.make_async_copy(w2_hbm, w2_buf, w2_sem.at[0])

        def b1_copy():
            return pltpu.make_async_copy(b1_hbm, b1_buf, b_sem.at[0])

        def b2_copy():
            return pltpu.make_async_copy(b2_hbm, b2_buf, b_sem.at[1])

        def o_copy(rb, cb):
            rows = pl.ds(rb * _ROW_CHUNK, _ROW_CHUNK)
            cols = pl.ds(cb * _LANE, _LANE)
            return pltpu.make_async_copy(
                o_buf.at[rows, cols], o_hbm.at[rows, cols], o_sem.at[0])

        b1_copy().start()
        b2_copy().start()
        w1_copy(0).start()
        x_copy(0).start()
        x_copy(1).start()
        for c in range(1, n_w1):
            w1_copy(c).start()
        x_copy(2).start()
        w2_copy().start()

        x_copy(0).wait()
        b1_copy().wait()
        b1 = b1_buf[...].reshape(1, F).astype(jnp.float32)

        def a_block(r0, r1, c0, c1):
            h = lax.dot_general(x_buf[r0:r1, :], w1_buf[c0:c1, :], _NT,
                                preferred_element_type=jnp.float32)
            g_buf[r0:r1, c0:c1] = _gelu_tanh(h + b1[:, c0:c1]).astype(jnp.bfloat16)

        for c in range(n_w1):
            c0, c1 = w1_bounds[c], min(w1_bounds[c + 1], f_main)
            w1_copy(c).wait()
            if c == 0:
                a_block(*x_rows[0], c0, c1)
                x_copy(1).wait()
                a_block(*x_rows[1], c0, c1)
            else:
                a_block(0, r_early, c0, c1)

        x_copy(2).wait()
        if F > f_main:
            ht = lax.dot_general(w1_buf[f_main:F, :], x_buf[...], _NT,
                                 preferred_element_type=jnp.float32)
            g_buf[:, f_main:F] = _gelu_tanh(
                ht.T + b1[:, f_main:F]).astype(jnp.bfloat16)
        r0 = r_early
        for rows in rest_chunks:
            a_block(r0, r0 + rows, 0, f_main)
            r0 += rows
        assert r0 == M

        w2_copy().wait()
        b2_copy().wait()
        b2 = b2_buf[...].reshape(1, D).astype(jnp.float32)
        for cb in range(n_cb):
            n0 = cb * _LANE
            for rb in range(n_rb):
                r0 = rb * _ROW_CHUNK
                o = jnp.dot(g_buf[r0:r0 + _ROW_CHUNK, :], w2_buf[:, n0:n0 + _LANE],
                            preferred_element_type=jnp.float32)
                o_buf[r0:r0 + _ROW_CHUNK, n0:n0 + _LANE] = (
                    o + b2[:, n0:n0 + _LANE]).astype(o_buf.dtype)
                o_copy(rb, cb).start()

        for cb in range(n_cb):
            for rb in range(n_rb):
                o_copy(rb, cb).wait()

    scratch = [
        pltpu.VMEM((M, D), jnp.bfloat16),
        pltpu.VMEM((F, D), jnp.bfloat16),
        pltpu.VMEM((F, D), jnp.bfloat16),
        pltpu.VMEM((F,), jnp.bfloat16),
        pltpu.VMEM((D,), jnp.bfloat16),
        pltpu.VMEM((M, F), jnp.bfloat16),
        pltpu.VMEM((M, D), jnp.bfloat16),
        pltpu.SemaphoreType.DMA((n_x,)),
        pltpu.SemaphoreType.DMA((n_w1,)),
        pltpu.SemaphoreType.DMA((1,)),
        pltpu.SemaphoreType.DMA((2,)),
        pltpu.SemaphoreType.DMA((1,)),
    ]
    return kernel, scratch


@jax.jit
def pallas_standalone__dense_activation_gelu__prompt_kernel(
    x: jax.Array,
    w1: jax.Array,
    b1: jax.Array,
    w2: jax.Array,
    b2: jax.Array,
):
    B, S, D = x.shape
    F = w1.shape[1]
    M = B * S
    kernel, scratch = _make_kernel(M, D, F)
    any_spec = pl.BlockSpec(memory_space=pl.ANY)
    out = pl.pallas_call(
        kernel,
        in_specs=[any_spec] * 5,
        out_specs=any_spec,
        out_shape=jax.ShapeDtypeStruct((M, D), x.dtype),
        scratch_shapes=scratch,
        compiler_params=pltpu.CompilerParams(
            vmem_limit_bytes=64 * 1024 * 1024,
        ),
    )(x.reshape(M, D), w1.T, b1, w2, b2)
    return out.reshape(B, S, D)
```
